```python
import jax
import jax.numpy as jnp

def _softmax(x, axis=-1):
    return jax.nn.softmax(x, axis=axis)
def _gelu(x):
    return jax.nn.gelu(x, approximate=True)
def _silu(x):
    return jax.nn.silu(x)
def _sigmoid(x):
    return jax.nn.sigmoid(x)
def _layernorm(x, axis=-1, eps=1e-5):
    m = jnp.mean(x, axis=axis, keepdims=True)
    v = jnp.var(x, axis=axis, keepdims=True)
    return (x - m) / jnp.sqrt(v + eps)
def _scatter_add(tgt, idx, src, axis=0):
    return tgt.at[idx].add(src)
def _segment_sum(src, seg, n):
    return jax.ops.segment_sum(src, seg, n)
class _Rng:
    def __init__(self, key):
        self._k = key
    def _next(self):
        self._k, sub = jax.random.split(self._k)
        return sub
    def normal(self, shape):
        return jax.random.normal(self._next(), shape, dtype=jnp.bfloat16)
    def randint(self, lo, hi, shape):
        return jax.random.randint(self._next(), shape, lo, hi, dtype=jnp.int32)
    def uniform(self, shape, lo=0.0, hi=1.0):
        return jax.random.uniform(self._next(), shape, jnp.bfloat16, lo, hi)
    def permutation(self, n):
        return jax.random.permutation(self._next(), n)


kernel_name = 'gated_mix__compressed_kv_cla__ssm_conv_s5__prompt'

def setup_inputs():
    _rng = _Rng(jax.random.key(int.from_bytes(__import__("os").urandom(4), "little")))
    _w = (lambda a: (lambda t: t.astype(jnp.bfloat16) if jnp.issubdtype(t.dtype, jnp.floating) else t)(jnp.asarray(a)))
    def _A_setup():
        B, H, Sq, Sk, D, M = 1, 16, 2048, 2048, 256, 448
        Dc = 4 * D
        return {
            "x": _w((lambda *s: _rng.normal(s) * 0.05)(B, Sq, M)),
            "c_kv": _w((lambda *s: _rng.normal(s) * 0.05)(B, Sk, Dc)),
            "w_q": _w((lambda *s: _rng.normal(s) * 0.05)(M, H, D) * (M ** -0.5)),
            "w_uk": _w((lambda *s: _rng.normal(s) * 0.05)(Dc, H, D) * (Dc ** -0.5)),
            "w_uv": _w((lambda *s: _rng.normal(s) * 0.05)(Dc, H, D) * (Dc ** -0.5)),
            "w_o": _w((lambda *s: _rng.normal(s) * 0.05)(H, D, M) * ((H * D) ** -0.5)),
        }
    _A_in = _A_setup()

    def _B_setup():
        B, S, D = 1, 2048, 448
        P = D
        Lambda_re = -0.5 * jnp.exp((lambda *s: _rng.normal(s) * 0.05)(P))
        Lambda_im = (lambda *s: _rng.normal(s) * 0.05)(P) * 1.0
        B_re = (lambda *s: _rng.normal(s) * 0.05)(P, D) * (D ** -0.5)
        B_im = (lambda *s: _rng.normal(s) * 0.05)(P, D) * (D ** -0.5)
        C_re = (lambda *s: _rng.normal(s) * 0.05)(D, P) * (P ** -0.5)
        C_im = (lambda *s: _rng.normal(s) * 0.05)(D, P) * (P ** -0.5)
        log_dt = (lambda *s: _rng.normal(s) * 0.05)(P) * 0.3 - 2.0
        Dskip = (lambda *s: _rng.normal(s) * 0.05)(D)
        return {
            "x": _w((lambda *s: _rng.normal(s) * 0.05)(B, S, D)),
            "Lambda_re": _w(Lambda_re),
            "Lambda_im": _w(Lambda_im),
            "B_re": _w(B_re),
            "B_im": _w(B_im),
            "C_re": _w(C_re),
            "C_im": _w(C_im),
            "log_dt": _w(log_dt),
            "Dskip": _w(Dskip),
        }
    _B_in = _B_setup()

    return {
        "A_x": _A_in["x"],
        "A_c_kv": _A_in["c_kv"],
        "A_w_q": _A_in["w_q"],
        "A_w_uk": _A_in["w_uk"],
        "A_w_uv": _A_in["w_uv"],
        "A_w_o": _A_in["w_o"],
        "B_x": _B_in["x"],
        "B_Lambda_re": _B_in["Lambda_re"],
        "B_Lambda_im": _B_in["Lambda_im"],
        "B_B_re": _B_in["B_re"],
        "B_B_im": _B_in["B_im"],
        "B_C_re": _B_in["C_re"],
        "B_C_im": _B_in["C_im"],
        "B_log_dt": _B_in["log_dt"],
        "B_Dskip": _B_in["Dskip"],
        "gate_w": _w((lambda *s: _rng.normal(s) * 0.05)(448)),
    }

def reference(A_x, A_c_kv, A_w_q, A_w_uk, A_w_uv, A_w_o, B_x, B_Lambda_re, B_Lambda_im, B_B_re, B_B_im, B_C_re, B_C_im, B_log_dt, B_Dskip, gate_w):
    def _A_ref(x, c_kv, w_q, w_uk, w_uv, w_o):
        B, Sq, M = x.shape[0], x.shape[1], x.shape[2]
        Sk = c_kv.shape[1]
        H, D = w_q.shape[1], w_q.shape[2]
        q = jnp.einsum("bqm,mhd->bhqd", x, w_q)
        k = jnp.einsum("bkc,chd->bhkd", c_kv, w_uk)
        v = jnp.einsum("bkc,chd->bhkd", c_kv, w_uv)
        scores = jnp.einsum("bhqd,bhkd->bhqk", q, k) * (D ** -0.5)
        off = Sk - Sq
        qi = jnp.arange(Sq)[:, None]
        kj = jnp.arange(Sk)[None, :]
        cmask = kj <= (qi + off)
        scores = jnp.where(cmask[None, None], scores, -1e9)
        p = _softmax(scores, axis=-1)
        ctx = jnp.einsum("bhqk,bhkd->bhqd", p, v)
        return jnp.einsum("bhqd,hdm->bqm", ctx, w_o)

    def _B_ref(x, Lambda_re, Lambda_im, B_re, B_im, C_re, C_im, log_dt, Dskip):
        Bsz, L, H = x.shape
        Lam = Lambda_re + 1j * Lambda_im
        Bmat = B_re + 1j * B_im
        Cmat = C_re + 1j * C_im
        dt = jnp.exp(log_dt)
        Lam_bar = jnp.exp(dt * Lam)
        B_bar = ((Lam_bar - 1.0) / Lam)[:, None] * Bmat
        Bu = jnp.einsum("bld,pd->blp", x + 0j, B_bar)
        h = jnp.zeros_like(Bu[:, 0, :])
        hs = []
        for t in range(L):
            h = Lam_bar[None, :] * h + Bu[:, t, :]
            hs.append(h)
        hseq = jnp.stack(hs, 1)
        y = 2.0 * jnp.einsum("blp,dp->bld", hseq, Cmat).real + x * Dskip[None, None, :]
        return y

    x = A_x
    g = _sigmoid((x * gate_w).sum(-1, keepdims=True))
    a = _A_ref(x, A_c_kv, A_w_q, A_w_uk, A_w_uv, A_w_o)
    b = _B_ref(x, B_Lambda_re, B_Lambda_im, B_B_re, B_B_im, B_C_re, B_C_im, B_log_dt, B_Dskip)
    return g * a + (1 - g) * b
```

```python
import functools

import jax
import jax.numpy as jnp
import numpy as np
import jax.experimental.pallas as pl
import jax.experimental.pallas.tpu as pltpu

F32 = jnp.float32
BF16 = jnp.bfloat16
LOG2E = float(np.log2(np.e))
NT = (((1,), (1,)), ((), ()))
TQ = 256
TP = 1024
TS = 512
TSS = 128
AHEAD = 3


def _dot(a, b):
    return jnp.dot(a, b, preferred_element_type=F32)


def _dot_nt(a, b):
    return jax.lax.dot_general(a, b, NT, preferred_element_type=F32)


def _cmul(ar, ai, br, bi):
    return ar * br - ai * bi, ar * bi + ai * br


def _col(ref):
    v = ref[...].astype(F32).reshape(1, -1)
    return jnp.broadcast_to(v, (128, v.shape[1])).T


def _ssm(xt_ref, lre_ref, lim_ref, bre_ref, bim_ref, cre_ref, cim_ref, ldt_ref,
         dsk_ref, o_ref, x_ref, acc_ref):
    S, P = x_ref.shape
    T = TSS
    ld = lambda r: r[...].astype(F32).reshape(1, -1)
    lre = ld(lre_ref)
    lim = ld(lim_ref)
    dt = jnp.exp(ld(ldt_ref)).astype(BF16).astype(F32)
    mag = jnp.exp(dt * lre)
    ar = mag * jnp.cos(dt * lim)
    ai = mag * jnp.sin(dt * lim)
    den = lre * lre + lim * lim
    cr, ci = _cmul(ar - 1.0, ai, lre / den, -lim / den)
    row = jax.lax.broadcasted_iota(jnp.int32, (8, P), 0)
    b = lambda t: jnp.broadcast_to(t, (8, P))
    pw = [(ar, ai)]
    for _ in range(7):
        pw.append(_cmul(pw[-1][0], pw[-1][1], ar, ai))
    steps = []
    for d in (1, 2, 4):
        steps.append((d, jnp.where(row >= d, b(pw[d - 1][0]), 0.0),
                      jnp.where(row >= d, b(pw[d - 1][1]), 0.0)))
    tr = b(pw[0][0])
    ti = b(pw[0][1])
    for s in range(1, 8):
        tr = jnp.where(row == s, b(pw[s][0]), tr)
        ti = jnp.where(row == s, b(pw[s][1]), ti)
    cr = b(cr)
    ci = b(ci)
    dsk = _col(dsk_ref)

    def scan(u_re, u_im, carry):
        pr, pi_ = carry
        outr, outi = [], []
        for a in range(0, u_re.shape[0], 8):
            ur, ui = _cmul(u_re[a:a + 8], u_im[a:a + 8], cr, ci)
            for d, mr, mi in steps:
                dr, di = _cmul(pltpu.roll(ur, d, 0), pltpu.roll(ui, d, 0), mr, mi)
                ur, ui = ur + dr, ui + di
            dr, di = _cmul(b(pr[7:8, :]), b(pi_[7:8, :]), tr, ti)
            pr, pi_ = ur + dr, ui + di
            outr.append(pr)
            outi.append(pi_)
        return (jnp.concatenate(outr, 0).astype(BF16), jnp.concatenate(outi, 0).astype(BF16),
                (pr, pi_))

    def chunk(n, carry):
        us = []
        for j in range(TS // T):
            sl = pl.ds(pl.multiple_of(n * TS + j * T, T), T)
            x = xt_ref[:, sl].astype(F32).T.astype(BF16)
            x_ref[sl, :] = x
            acc_ref[:, sl] = jnp.zeros((acc_ref.shape[0], T), F32)
            us.append((sl, _dot_nt(x, bre_ref[...]), _dot_nt(x, bim_ref[...])))
        for sl, u_re, u_im in us:
            hr, hi, carry = scan(u_re, u_im, carry)
            y = _dot_nt(cre_ref[...], hr) - _dot_nt(cim_ref[...], hi)
            o_ref[:, sl] = 2.0 * y + xt_ref[:, sl].astype(F32) * jnp.tile(dsk, (1, T // 128))
        return carry

    z = jnp.zeros((8, P), F32)
    jax.lax.fori_loop(0, S // TS, chunk, (z, z))


def _kernel(xt_ref, c_hbm, wq_hbm, wk_hbm, wv_hbm, wot_ref,
            lre_ref, lim_ref, bre_ref, bim_ref, cre_ref, cim_ref, ldt_ref, dsk_ref, gw_ref,
            o_ref,
            wq_buf, wk_buf, wv_buf, sems, c_ref, csem, x_ref, q_ref, k_ref, v_ref, acc_ref):
    h = pl.program_id(0)
    nh = pl.num_programs(0)
    S, M = x_ref.shape
    D = q_ref.shape[1]
    pair = h // 2
    slot = pair % 2

    def copies(j, s):
        return [
            pltpu.make_async_copy(w.bitcast(jnp.uint32).at[:, j, :], buf.at[s], sems.at[n, s])
            for n, (w, buf) in enumerate(((wq_hbm, wq_buf), (wk_hbm, wk_buf), (wv_hbm, wv_buf)))
        ]

    @pl.when(h == 0)
    def _():
        ccp = pltpu.make_async_copy(c_hbm.at[0], c_ref, csem)
        ccp.start()
        for cp in copies(0, 0):
            cp.start()
        _ssm(xt_ref, lre_ref, lim_ref, bre_ref, bim_ref, cre_ref, cim_ref, ldt_ref,
             dsk_ref, o_ref, x_ref, acc_ref)
        ccp.wait()

    @pl.when(h % 2 == 0)
    def _():
        @pl.when(h + 2 < nh)
        def _():
            for cp in copies(pair + 1, 1 - slot):
                cp.start()
        for cp in copies(pair, slot):
            cp.wait()

    sh = ((1 - h % 2) * 16).astype(jnp.uint32)

    def unpack(buf):
        w = (buf[slot] << sh) & jnp.uint32(0xFFFF0000)
        return pltpu.bitcast(w, F32).astype(BF16)

    def proj(i, _):
        sl = pl.ds(pl.multiple_of(i * TP, TP), TP)
        q_ref[sl, :] = (_dot(x_ref[sl, :], unpack(wq_buf)) * (LOG2E * D ** -0.5)).astype(BF16)
        k_ref[sl, :] = _dot(c_ref[sl, :], unpack(wk_buf)).astype(BF16)
        v_ref[sl, :] = _dot(c_ref[sl, :], unpack(wv_buf)).astype(BF16)

    jax.lax.fori_loop(0, S // TP, proj, None)

    NEG = -1e9 * LOG2E
    HB = 128
    tri = (jax.lax.broadcasted_iota(jnp.int32, (HB, HB), 1)
           <= jax.lax.broadcasted_iota(jnp.int32, (HB, HB), 0))
    nq = S // HB

    def qk(i):
        return _dot_nt(q_ref[i * HB:(i + 1) * HB, :], k_ref[0:(i + 1) * HB, :])

    def attend(i, s):
        d = jnp.where(tri, s[:, i * HB:], NEG)
        s = jnp.concatenate([s[:, 0:i * HB], d], axis=1) if i else d
        p = jnp.exp2(s - jnp.max(s, axis=1, keepdims=True))
        inv = 1.0 / jnp.sum(p, axis=1, keepdims=True)
        return (_dot(p.astype(BF16), v_ref[0:(i + 1) * HB, :]) * inv).astype(BF16)

    order = list(range(nq))
    sc, cs = {}, {}
    for n in range(nq + AHEAD + 2):
        if n < nq:
            sc[order[n]] = qk(order[n])
        m = n - AHEAD
        if m >= 3 and m % 2 == 1:
            j = min(order[m - 3], order[m - 2])
            ctx = jnp.concatenate([cs.pop(j), cs.pop(j + 1)], axis=0)
            acc_ref[:, j * HB:(j + 2) * HB] += _dot_nt(wot_ref[0], ctx)
        if 0 <= m < nq:
            cs[order[m]] = attend(order[m], sc.pop(order[m]))

    @pl.when(h == nh - 1)
    def _():
        gw = jnp.broadcast_to(gw_ref[...].astype(F32).reshape(1, -1), (16, M)).astype(BF16)

        def fin(n, _):
            sl = pl.ds(pl.multiple_of(n * TQ, TQ), TQ)
            g = jax.nn.sigmoid(_dot(gw, xt_ref[:, sl])[0:1, :])
            o_ref[:, sl] = g * acc_ref[:, sl] + (1.0 - g) * o_ref[:, sl]

        jax.lax.fori_loop(0, S // TQ, fin, None)


@jax.jit
def pallas_gated_mix__compressed_kv_cla__ssm_conv_s5__prompt_kernel(
    A_x, A_c_kv, A_w_q, A_w_uk, A_w_uv, A_w_o, B_x, B_Lambda_re, B_Lambda_im,
    B_B_re, B_B_im, B_C_re, B_C_im, B_log_dt, B_Dskip, gate_w,
):
    del B_x
    _, S, M = A_x.shape
    Dc = A_c_kv.shape[2]
    _, H, D = A_w_q.shape
    P = B_Lambda_re.shape[0]
    full = lambda t: pl.BlockSpec(t.shape, lambda h: (0,) * t.ndim)
    anyspec = pl.BlockSpec(memory_space=pltpu.HBM)
    xt = A_x[0].T
    wot = jnp.swapaxes(A_w_o, 1, 2)
    small = [B_Lambda_re, B_Lambda_im, B_B_re, B_B_im, B_C_re, B_C_im,
             B_log_dt, B_Dskip, gate_w]
    out_t = pl.pallas_call(
        _kernel,
        grid=(H,),
        in_specs=[full(xt), anyspec, anyspec, anyspec, anyspec,
                  pl.BlockSpec((1, M, D), lambda h: (h, 0, 0))] + [full(t) for t in small],
        out_specs=pl.BlockSpec((M, S), lambda h: (0, 0)),
        out_shape=jax.ShapeDtypeStruct((M, S), F32),
        scratch_shapes=[
            pltpu.VMEM((2, M, D), jnp.uint32),
            pltpu.VMEM((2, Dc, D), jnp.uint32),
            pltpu.VMEM((2, Dc, D), jnp.uint32),
            pltpu.SemaphoreType.DMA((3, 2)),
            pltpu.VMEM((S, Dc), BF16),
            pltpu.SemaphoreType.DMA,
            pltpu.VMEM((S, M), BF16),
            pltpu.VMEM((S, D), BF16),
            pltpu.VMEM((S, D), BF16),
            pltpu.VMEM((S, D), BF16),
            pltpu.VMEM((M, S), F32),
        ],
        compiler_params=pltpu.CompilerParams(
            dimension_semantics=("arbitrary",), vmem_limit_bytes=110 << 20),
    )(xt, A_c_kv, A_w_q, A_w_uk, A_w_uv, wot, *small)
    return out_t.T[None]
```
